```python
import os as _os
_os.environ.setdefault("JAX_PLATFORMS", "cpu")
import jax
import jax.numpy as jnp

def _softmax(x, axis=-1):
    return jax.nn.softmax(x, axis=axis)
def _gelu(x):
    return jax.nn.gelu(x, approximate=True)
def _silu(x):
    return jax.nn.silu(x)
def _sigmoid(x):
    return jax.nn.sigmoid(x)
def _layernorm(x, axis=-1, eps=1e-5):
    m = jnp.mean(x, axis=axis, keepdims=True)
    v = jnp.var(x, axis=axis, keepdims=True)
    return (x - m) / jnp.sqrt(v + eps)
def _scatter_add(tgt, idx, src, axis=0):
    return tgt.at[idx].add(src)
def _segment_sum(src, seg, n):
    return jax.ops.segment_sum(src, seg, n)
class _Rng:
    def __init__(self, key):
        self._k = key
    def _next(self):
        self._k, sub = jax.random.split(self._k)
        return sub
    def normal(self, shape):
        return jax.random.normal(self._next(), shape, dtype=jnp.bfloat16)
    def randint(self, lo, hi, shape):
        return jax.random.randint(self._next(), shape, lo, hi, dtype=jnp.int32)
    def uniform(self, shape, lo=0.0, hi=1.0):
        return jax.random.uniform(self._next(), shape, jnp.bfloat16, lo, hi)
    def permutation(self, n):
        return jax.random.permutation(self._next(), n)


kernel_name = 'concat_heads__mha_block_cached__mha_block_cached__near_ridge'

def setup_inputs():
    _rng = _Rng(jax.random.key(int.from_bytes(__import__("os").urandom(4), "little")))
    _w = (lambda a: (lambda t: t.astype(jnp.bfloat16) if jnp.issubdtype(t.dtype, jnp.floating) else t)(jnp.asarray(a)))
    def _A_setup():
        B, Sq, D = 32, 32, 640
        H, Sk, Dh = 32, 32, 128
        return {
            "x": _w((lambda *s: _rng.normal(s) * 0.8)(B, Sq, D)),
            "k_cache": _w((lambda *s: _rng.normal(s) * 0.8)(B, H, Sk, Dh)),
            "v_cache": _w((lambda *s: _rng.normal(s) * 0.05)(B, H, Sk, Dh)),
            "wq": _w((lambda *s: _rng.normal(s) * 0.8)(D, H * Dh) * (D ** -0.5)),
            "wo": _w((lambda *s: _rng.normal(s) * 0.05)(H * Dh, D) * ((H * Dh) ** -0.5)),
        }
    _A_in = _A_setup()

    def _B_setup():
        B, Sq, D = 32, 32, 640
        H, Sk, Dh = 32, 32, 128
        return {
            "x": _w((lambda *s: _rng.normal(s) * 0.8)(B, Sq, D)),
            "k_cache": _w((lambda *s: _rng.normal(s) * 0.8)(B, H, Sk, Dh)),
            "v_cache": _w((lambda *s: _rng.normal(s) * 0.05)(B, H, Sk, Dh)),
            "wq": _w((lambda *s: _rng.normal(s) * 0.8)(D, H * Dh) * (D ** -0.5)),
            "wo": _w((lambda *s: _rng.normal(s) * 0.05)(H * Dh, D) * ((H * Dh) ** -0.5)),
        }
    _B_in = _B_setup()

    return {
        "A_x": _A_in["x"],
        "A_k_cache": _A_in["k_cache"],
        "A_v_cache": _A_in["v_cache"],
        "A_wq": _A_in["wq"],
        "A_wo": _A_in["wo"],
        "B_x": _B_in["x"],
        "B_k_cache": _B_in["k_cache"],
        "B_v_cache": _B_in["v_cache"],
        "B_wq": _B_in["wq"],
        "B_wo": _B_in["wo"],
    }

def reference(A_x, A_k_cache, A_v_cache, A_wq, A_wo, B_x, B_k_cache, B_v_cache, B_wq, B_wo):
    def _A_ref(x, k_cache, v_cache, wq, wo):
        B, Sq, D = x.shape
        H, Dh = 32, 128
        q = (lambda x, *d: x.transpose(*d))((x @ wq).reshape(B, Sq, H, Dh), 0, 2, 1, 3)
        scores = jnp.einsum("bhqd,bhkd->bhqk", q, k_cache) * (Dh ** -0.5)
        p = _softmax(scores, axis=-1)
        o = jnp.einsum("bhqk,bhkd->bhqd", p, v_cache)
        return (lambda x, *d: x.transpose(*d))(o, 0, 2, 1, 3).reshape(B, Sq, H * Dh) @ wo

    def _B_ref(x, k_cache, v_cache, wq, wo):
        B, Sq, D = x.shape
        H, Dh = 32, 128
        q = (lambda x, *d: x.transpose(*d))((x @ wq).reshape(B, Sq, H, Dh), 0, 2, 1, 3)
        scores = jnp.einsum("bhqd,bhkd->bhqk", q, k_cache) * (Dh ** -0.5)
        p = _softmax(scores, axis=-1)
        o = jnp.einsum("bhqk,bhkd->bhqd", p, v_cache)
        return (lambda x, *d: x.transpose(*d))(o, 0, 2, 1, 3).reshape(B, Sq, H * Dh) @ wo

    a = _A_ref(A_x, A_k_cache, A_v_cache, A_wq, A_wo)
    b = _B_ref(B_x, B_k_cache, B_v_cache, B_wq, B_wo)
    return jnp.concatenate([a, b], axis=-1)
```

```python
import jax
import jax.numpy as jnp
from jax import lax
from jax.experimental import pallas as pl
from jax.experimental.pallas import tpu as pltpu

NB, SQ, D, H, SK, DH = 32, 32, 640, 32, 32, 128
M = NB * SQ
HB = 4
NS = H // HB
NG = NB // 4
SCALE = DH ** -0.5
F32, BF16, U32 = jnp.float32, jnp.bfloat16, jnp.uint32
X_CHUNKS = (((0, 256), (256, 256), (512, 512)), ((0, 512), (512, 512)))
OUT_CHUNKS = ((0, 384), (384, 384), (768, 128), (896, 128))


def _kernel(xa, ka, va, wqa, woa, xb, kb, vb, wqb, wob, out_hbm,
            xs0, xs1, kbuf0, kbuf1, vbuf0, vbuf1, wqbuf0, wqbuf1, wobuf0, wobuf1,
            qs0, qs1, os0, os1, acc0, acc1, ost0, ost1, s_scr, p_scr, xsem, sem, osem):
    srcs = ((xa, ka, va, wqa, woa), (xb, kb, vb, wqb, wob))
    xs, kbuf, vbuf, wqbuf, wobuf = (xs0, xs1), (kbuf0, kbuf1), (vbuf0, vbuf1), (wqbuf0, wqbuf1), (wobuf0, wobuf1)
    qs, os_, acc, ostage = (qs0, qs1), (os0, os1), (acc0, acc1), (ost0, ost1)
    lane = lax.broadcasted_iota(jnp.int32, (SK, 128), 1)
    lane16 = lax.broadcasted_iota(jnp.int32, (SK // 2, 128), 1)

    def x_copy(br, c):
        r = pl.ds(*X_CHUNKS[br][c])
        return pltpu.make_async_copy(srcs[br][0].at[r, :], xs[br].at[r, :], xsem.at[br, c])

    def cp(kind, br, i):
        _, k, v, wq, wo = srcs[br]
        cols = pl.ds(pl.multiple_of(i * (HB * DH), HB * DH), HB * DH)
        heads = pl.ds(i * HB, HB)
        if kind == 'q':
            return pltpu.make_async_copy(wq.at[:, cols], wqbuf[br], sem.at[br, 0])
        if kind == 'k':
            return pltpu.make_async_copy(k.at[:, heads], kbuf[br], sem.at[br, 1])
        if kind == 'v':
            return pltpu.make_async_copy(v.at[:, heads], vbuf[br], sem.at[br, 2])
        return pltpu.make_async_copy(wo.at[cols, :], wobuf[br], sem.at[br, 3])

    def out_copy(br, c):
        r = pl.ds(*OUT_CHUNKS[c])
        return pltpu.make_async_copy(ostage[br].at[r, :], out_hbm.at[r, pl.ds(br * D, D)], osem.at[br, c])

    def qproj(br, r0=0, n=M):
        q = jnp.dot(xs[br][r0:r0 + n, :], wqbuf[br][...], preferred_element_type=F32)
        for h in range(HB):
            qs[br][h, r0:r0 + n, :] = q[:, h * DH:(h + 1) * DH].astype(BF16)

    def scores(br):
        for h in range(HB):
            for g in range(NG):
                kg = kbuf[br][4 * g:4 * g + 4, h].reshape(128, DH)
                qg = qs[br][h, 128 * g:128 * g + 128, :]
                st = lax.dot_general(kg, qg, (((1,), (1,)), ((), ())), preferred_element_type=F32)
                s_scr[h, g] = jnp.where(lane < 32, st[0:32],
                                        jnp.where(lane < 64, st[32:64], jnp.where(lane < 96, st[64:96], st[96:128])))

    def softmax(br):
        for h in range(HB):
            for g in range(NG):
                c = s_scr[h, g]
                e = jnp.exp((c - jnp.max(c, axis=0, keepdims=True)) * SCALE)
                p = e * (1.0 / jnp.sum(e, axis=0, keepdims=True))
                p_scr[h, g] = pltpu.bitcast(p.astype(BF16), U32)

    def pv(br):
        for h in range(HB):
            for g in range(NG):
                p = p_scr[h, g]
                blocks = [jnp.where((lane16 >= 32 * j) & (lane16 < 32 * j + 32), p, jnp.uint32(0)) for j in range(4)]
                pt = pltpu.bitcast(jnp.concatenate(blocks, axis=0), BF16)
                vg = vbuf[br][4 * g:4 * g + 4, h].reshape(128, DH)
                o = lax.dot_general(pt, vg, (((0,), (0,)), ((), ())), preferred_element_type=F32)
                os_[br][h, 128 * g:128 * g + 128, :] = o.astype(BF16)

    def oproj(br, first=False, last=False):
        def contrib(r0, n):
            o = jnp.concatenate([os_[br][h, r0:r0 + n, :] for h in range(HB)], axis=1)
            return jnp.dot(o, wobuf[br][...], preferred_element_type=F32)
        if first:
            acc[br][...] = contrib(0, M)
        elif not last:
            acc[br][...] += contrib(0, M)
        else:
            for c, (r0, n) in enumerate(OUT_CHUNKS):
                ostage[br][r0:r0 + n, :] = (acc[br][r0:r0 + n, :] + contrib(r0, n)).astype(BF16)
                out_copy(br, c).start()

    def body(par, i, split_wait=False, first_o=False, last_o=False, start_q=True, final=False):
        oth = 1 - par
        i_next, i_prev = i + par, i - 1 + par

        def prefetch():
            cp('o', par, i).start()
            if not final:
                cp('k', oth, i_next).start()
                if start_q:
                    cp('q', par, i + 1).start()
                cp('v', oth, i_next).start()

        def wait_attention():
            cp('k', par, i).wait()
            cp('v', par, i).wait()
            if not final:
                cp('q', oth, i_next).wait()

        if split_wait:
            cp('o', oth, i_prev).wait()
            oproj(oth, first_o)
            prefetch()
            wait_attention()
        else:
            prefetch()
            cp('o', oth, i_prev).wait()
            wait_attention()
            oproj(oth, first_o, last_o)
        scores(par)
        if not final:
            qproj(oth)
        softmax(par)
        pv(par)

    groups = [
        [x_copy(0, 1), x_copy(0, 2)],
        [cp('q', 1, 0), x_copy(1, 0)],
        [x_copy(1, 1)],
        [cp('k', 0, 0)],
        [cp('v', 0, 0)],
    ]
    cp('q', 0, 0).start()
    x_copy(0, 0).start()
    for br in range(2):
        cp('q', br, 0).wait()
        for c, (r0, n) in enumerate(X_CHUNKS[br]):
            x_copy(br, c).wait()
            for d in groups.pop(0):
                d.start()
            qproj(br, r0, n)
            if br == 1:
                acc[1][r0:r0 + n, :] = jnp.zeros((n, D), F32)

    cp('o', 0, 0).start()
    cp('k', 1, 0).start()
    cp('q', 0, 1).start()
    cp('v', 1, 0).start()
    cp('k', 0, 0).wait()
    cp('v', 0, 0).wait()
    scores(0)
    softmax(0)
    pv(0)

    body(1, 0, split_wait=True, first_o=True)

    def pair(j, carry):
        body(0, j)
        body(1, j)
        return carry

    lax.fori_loop(1, NS - 1, pair, 0)
    body(0, NS - 1, start_q=False)
    body(1, NS - 1, last_o=True, final=True)
    cp('o', 1, NS - 1).wait()
    oproj(1, last=True)
    for br in range(2):
        for c in range(len(OUT_CHUNKS)):
            out_copy(br, c).wait()


@jax.jit
def pallas_concat_heads__mha_block_cached__mha_block_cached__near_ridge_kernel(
    A_x: jax.Array,
    A_k_cache: jax.Array,
    A_v_cache: jax.Array,
    A_wq: jax.Array,
    A_wo: jax.Array,
    B_x: jax.Array,
    B_k_cache: jax.Array,
    B_v_cache: jax.Array,
    B_wq: jax.Array,
    B_wo: jax.Array,
):
    hbm = pl.BlockSpec(memory_space=pl.ANY)
    vmem = pltpu.VMEM
    scratch = (
        [vmem((M, D), BF16)] * 2
        + [vmem((NB, HB, SK, DH), BF16)] * 4
        + [vmem((D, HB * DH), BF16)] * 2
        + [vmem((HB * DH, D), BF16)] * 2
        + [vmem((HB, M, DH), BF16)] * 4
        + [vmem((M, D), F32)] * 2
        + [vmem((M, D), BF16)] * 2
        + [vmem((HB, NG, SK, 128), F32), vmem((HB, NG, SK // 2, 128), U32)]
        + [pltpu.SemaphoreType.DMA((2, 3)), pltpu.SemaphoreType.DMA((2, 4)),
           pltpu.SemaphoreType.DMA((2, len(OUT_CHUNKS)))]
    )
    out = pl.pallas_call(
        _kernel,
        in_specs=[hbm] * 10,
        out_specs=hbm,
        out_shape=jax.ShapeDtypeStruct((M, 2 * D), BF16),
        scratch_shapes=scratch,
        compiler_params=pltpu.CompilerParams(vmem_limit_bytes=100 * 1024 * 1024),
    )(A_x.reshape(M, D), A_k_cache, A_v_cache, A_wq, A_wo, B_x.reshape(M, D), B_k_cache, B_v_cache, B_wq, B_wo)
    return out.reshape(NB, SQ, 2 * D)
```

```python
import jax
import jax.numpy as jnp
from jax import lax
from jax.experimental import pallas as pl
from jax.experimental.pallas import tpu as pltpu

NB, SQ, D, H, SK, DH = 32, 32, 640, 32, 32, 128
M = NB * SQ
HB = 4
NS = H // HB
NG = NB // 4
SCALE = DH ** -0.5
F32, BF16, U32 = jnp.float32, jnp.bfloat16, jnp.uint32
X_CHUNKS = (((0, 256), (256, 256), (512, 512)), ((0, 512), (512, 512)))
OUT_CH = (((0, 1024),), ((0, 384), (384, 384), (768, 128), (896, 128)))


def _kernel(xa, ka, va, wqa, woa, xb, kb, vb, wqb, wob, out_hbm,
            xs0, xs1, kbuf0, kbuf1, vbuf0, vbuf1, wqbuf0, wqbuf1, wobuf0, wobuf1,
            qs0, qs1, os0, os1, acc0, acc1, ost0, ost1, s_scr, p_scr, xsem, sem, osem):
    srcs = ((xa, ka, va, wqa, woa), (xb, kb, vb, wqb, wob))
    xs, kbuf, vbuf, wqbuf, wobuf = (xs0, xs1), (kbuf0, kbuf1), (vbuf0, vbuf1), (wqbuf0, wqbuf1), (wobuf0, wobuf1)
    qs, os_, acc, ostage = (qs0, qs1), (os0, os1), (acc0, acc1), (ost0, ost1)
    lane = lax.broadcasted_iota(jnp.int32, (SK, 128), 1)
    lane16 = lax.broadcasted_iota(jnp.int32, (SK // 2, 128), 1)

    def x_copy(br, c):
        r = pl.ds(*X_CHUNKS[br][c])
        return pltpu.make_async_copy(srcs[br][0].at[r, :], xs[br].at[r, :], xsem.at[br, c])

    def cp(kind, br, i):
        _, k, v, wq, wo = srcs[br]
        cols = pl.ds(pl.multiple_of(i * (HB * DH), HB * DH), HB * DH)
        heads = pl.ds(i * HB, HB)
        if kind == 'q':
            return pltpu.make_async_copy(wq.at[:, cols], wqbuf[br], sem.at[br, 0])
        if kind == 'k':
            return pltpu.make_async_copy(k.at[:, heads], kbuf[br], sem.at[br, 1])
        if kind == 'v':
            return pltpu.make_async_copy(v.at[:, heads], vbuf[br], sem.at[br, 2])
        return pltpu.make_async_copy(wo.at[cols, :], wobuf[br], sem.at[br, 3])

    def out_copy(br, c):
        r = pl.ds(*OUT_CH[br][c])
        return pltpu.make_async_copy(ostage[br].at[r, :], out_hbm.at[r, pl.ds(br * D, D)], osem.at[br, c])

    def qproj(br, r0=0, n=M):
        q = jnp.dot(xs[br][r0:r0 + n, :], wqbuf[br][...], preferred_element_type=F32)
        for h in range(HB):
            qs[br][h, r0:r0 + n, :] = q[:, h * DH:(h + 1) * DH].astype(BF16)

    def scores(br):
        for h in range(HB):
            for g in range(NG):
                kg = kbuf[br][4 * g:4 * g + 4, h].reshape(128, DH)
                qg = qs[br][h, 128 * g:128 * g + 128, :]
                st = lax.dot_general(kg, qg, (((1,), (1,)), ((), ())), preferred_element_type=F32)
                s_scr[h, g] = jnp.where(lane < 32, st[0:32],
                                        jnp.where(lane < 64, st[32:64], jnp.where(lane < 96, st[64:96], st[96:128])))

    def softmax(br):
        for h in range(HB):
            for g in range(NG):
                c = s_scr[h, g]
                e = jnp.exp((c - jnp.max(c, axis=0, keepdims=True)) * SCALE)
                p = e * (1.0 / jnp.sum(e, axis=0, keepdims=True))
                p_scr[h, g] = pltpu.bitcast(p.astype(BF16), U32)

    def pv(br):
        for h in range(HB):
            for g in range(NG):
                p = p_scr[h, g]
                blocks = [jnp.where((lane16 >= 32 * j) & (lane16 < 32 * j + 32), p, jnp.uint32(0)) for j in range(4)]
                pt = pltpu.bitcast(jnp.concatenate(blocks, axis=0), BF16)
                vg = vbuf[br][4 * g:4 * g + 4, h].reshape(128, DH)
                o = lax.dot_general(pt, vg, (((0,), (0,)), ((), ())), preferred_element_type=F32)
                os_[br][h, 128 * g:128 * g + 128, :] = o.astype(BF16)

    def oproj(br, first=False, last=False):
        def contrib(r0, n):
            o = jnp.concatenate([os_[br][h, r0:r0 + n, :] for h in range(HB)], axis=1)
            return jnp.dot(o, wobuf[br][...], preferred_element_type=F32)
        if first:
            acc[br][...] = contrib(0, M)
        elif not last:
            acc[br][...] += contrib(0, M)
        else:
            for c, (r0, n) in enumerate(OUT_CH[br]):
                ostage[br][r0:r0 + n, :] = (acc[br][r0:r0 + n, :] + contrib(r0, n)).astype(BF16)
                out_copy(br, c).start()

    def body(par, i, split_wait=False, first_o=False, last_o=False, start_q=True, final=False):
        oth = 1 - par
        i_next, i_prev = i + par, i - 1 + par

        def prefetch():
            cp('o', par, i).start()
            if not final:
                cp('k', oth, i_next).start()
                if start_q:
                    cp('q', par, i + 1).start()
                cp('v', oth, i_next).start()

        def wait_attention():
            cp('k', par, i).wait()
            cp('v', par, i).wait()
            if not final:
                cp('q', oth, i_next).wait()

        if split_wait:
            cp('o', oth, i_prev).wait()
            oproj(oth, first_o)
            prefetch()
            wait_attention()
        else:
            prefetch()
            cp('o', oth, i_prev).wait()
            wait_attention()
            oproj(oth, first_o, last_o)
        scores(par)
        if not final:
            qproj(oth)
        softmax(par)
        pv(par)

    groups = [
        [x_copy(0, 1), x_copy(0, 2)],
        [cp('q', 1, 0), x_copy(1, 0)],
        [x_copy(1, 1)],
        [cp('k', 0, 0)],
        [cp('v', 0, 0)],
    ]
    cp('q', 0, 0).start()
    x_copy(0, 0).start()
    for br in range(2):
        cp('q', br, 0).wait()
        for c, (r0, n) in enumerate(X_CHUNKS[br]):
            x_copy(br, c).wait()
            for d in groups.pop(0):
                d.start()
            qproj(br, r0, n)
            if br == 1:
                acc[1][r0:r0 + n, :] = jnp.zeros((n, D), F32)

    cp('o', 0, 0).start()
    cp('k', 1, 0).start()
    cp('q', 0, 1).start()
    cp('v', 1, 0).start()
    cp('k', 0, 0).wait()
    cp('v', 0, 0).wait()
    scores(0)
    softmax(0)
    pv(0)

    body(1, 0, split_wait=True, first_o=True)

    def pair(j, carry):
        body(0, j)
        body(1, j)
        return carry

    lax.fori_loop(1, NS - 1, pair, 0)
    body(0, NS - 1, start_q=False)
    body(1, NS - 1, last_o=True, final=True)
    cp('o', 1, NS - 1).wait()
    oproj(1, last=True)
    for br in range(2):
        for c in range(len(OUT_CH[br])):
            out_copy(br, c).wait()


@jax.jit
def pallas_concat_heads__mha_block_cached__mha_block_cached__near_ridge_kernel(
    A_x: jax.Array,
    A_k_cache: jax.Array,
    A_v_cache: jax.Array,
    A_wq: jax.Array,
    A_wo: jax.Array,
    B_x: jax.Array,
    B_k_cache: jax.Array,
    B_v_cache: jax.Array,
    B_wq: jax.Array,
    B_wo: jax.Array,
):
    hbm = pl.BlockSpec(memory_space=pl.ANY)
    vmem = pltpu.VMEM
    scratch = (
        [vmem((M, D), BF16)] * 2
        + [vmem((NB, HB, SK, DH), BF16)] * 4
        + [vmem((D, HB * DH), BF16)] * 2
        + [vmem((HB * DH, D), BF16)] * 2
        + [vmem((HB, M, DH), BF16)] * 4
        + [vmem((M, D), F32)] * 2
        + [vmem((M, D), BF16)] * 2
        + [vmem((HB, NG, SK, 128), F32), vmem((HB, NG, SK // 2, 128), U32)]
        + [pltpu.SemaphoreType.DMA((2, 3)), pltpu.SemaphoreType.DMA((2, 4)),
           pltpu.SemaphoreType.DMA((2, 4))]
    )
    out = pl.pallas_call(
        _kernel,
        in_specs=[hbm] * 10,
        out_specs=hbm,
        out_shape=jax.ShapeDtypeStruct((M, 2 * D), BF16),
        scratch_shapes=scratch,
        compiler_params=pltpu.CompilerParams(vmem_limit_bytes=100 * 1024 * 1024),
    )(A_x.reshape(M, D), A_k_cache, A_v_cache, A_wq, A_wo, B_x.reshape(M, D), B_k_cache, B_v_cache, B_wq, B_wo)
    return out.reshape(NB, SQ, 2 * D)
```
